```python
import os as _os
_os.environ.setdefault("JAX_PLATFORMS", "cpu")
import jax
import jax.numpy as jnp

def _softmax(x, axis=-1):
    return jax.nn.softmax(x, axis=axis)
def _gelu(x):
    return jax.nn.gelu(x, approximate=True)
def _silu(x):
    return jax.nn.silu(x)
def _sigmoid(x):
    return jax.nn.sigmoid(x)
def _layernorm(x, axis=-1, eps=1e-5):
    m = jnp.mean(x, axis=axis, keepdims=True)
    v = jnp.var(x, axis=axis, keepdims=True)
    return (x - m) / jnp.sqrt(v + eps)
def _scatter_add(tgt, idx, src, axis=0):
    return tgt.at[idx].add(src)
def _segment_sum(src, seg, n):
    return jax.ops.segment_sum(src, seg, n)
class _Rng:
    def __init__(self, key):
        self._k = key
    def _next(self):
        self._k, sub = jax.random.split(self._k)
        return sub
    def normal(self, shape):
        return jax.random.normal(self._next(), shape, dtype=jnp.bfloat16)
    def randint(self, lo, hi, shape):
        return jax.random.randint(self._next(), shape, lo, hi, dtype=jnp.int32)
    def uniform(self, shape, lo=0.0, hi=1.0):
        return jax.random.uniform(self._next(), shape, jnp.bfloat16, lo, hi)
    def permutation(self, n):
        return jax.random.permutation(self._next(), n)


kernel_name = 'concat_heads__sliding_local_dilated__linear_attn_block__prompt'

def setup_inputs():
    _rng = _Rng(jax.random.key(int.from_bytes(__import__("os").urandom(4), "little")))
    _w = (lambda a: (lambda t: t.astype(jnp.bfloat16) if jnp.issubdtype(t.dtype, jnp.floating) else t)(jnp.asarray(a)))
    def _A_setup():
        B, S, D = 1, 2048, 640
        return {
            "x": _w((lambda *s: _rng.normal(s) * 0.2)(B, S, D)),
            "wqkv": _w((lambda *s: _rng.normal(s) * 0.2)(D, 3 * D)),
            "wo": _w((lambda *s: _rng.normal(s) * 0.05)(D, D)),
        }
    _A_in = _A_setup()

    def _B_setup():
        B, S, D = 1, 2048, 640
        return {
            "x": _w((lambda *s: _rng.normal(s) * 0.05)(B, S, D)),
            "wqkv": _w((lambda *s: _rng.normal(s) * 1.6)(D, 3 * D)),
            "wo": _w((lambda *s: _rng.normal(s) * 0.4)(D, D)),
        }
    _B_in = _B_setup()

    return {
        "A_x": _A_in["x"],
        "A_wqkv": _A_in["wqkv"],
        "A_wo": _A_in["wo"],
        "B_x": _B_in["x"],
        "B_wqkv": _B_in["wqkv"],
        "B_wo": _B_in["wo"],
    }

def reference(A_x, A_wqkv, A_wo, B_x, B_wqkv, B_wo):
    def _A_ref(x, wqkv, wo):
        B, S, D = x.shape
        H = 32; Dh = D // H
        W, dil = 8, 2
        qkv = (lambda x, *d: x.transpose(*d))((x @ wqkv).reshape(B, S, 3, H, Dh), 2, 0, 3, 1, 4)
        q, k, v = qkv[0], qkv[1], qkv[2]
        scale = Dh ** -0.5
        pos = jnp.arange(S)
        off = jnp.arange(W) * dil
        idx = pos[:, None] - off[None, :]
        mask = idx >= 0
        idx_c = jnp.where(mask, idx, 0).reshape(-1)
        kg = k[:, :, idx_c, :].reshape(B, H, S, W, Dh)
        vg = v[:, :, idx_c, :].reshape(B, H, S, W, Dh)
        logits = jnp.einsum("bhsd,bhswd->bhsw", q, kg) * scale
        logits = jnp.where(mask[None, None, :, :], logits, -1e9)
        attn = _softmax(logits, axis=-1)
        o = jnp.einsum("bhsw,bhswd->bhsd", attn, vg)
        return (lambda x, *d: x.transpose(*d))(o, 0, 2, 1, 3).reshape(B, S, D) @ wo

    def _B_ref(x, wqkv, wo):
        B, S, D = x.shape
        H = 32; Dh = D // H
        qkv = (lambda x, *d: x.transpose(*d))((x @ wqkv).reshape(B, S, 3, H, Dh), 2, 0, 3, 1, 4)
        q, k, v = qkv[0], qkv[1], qkv[2]
        phi = lambda t: jnp.where(t > 0, t + 1, jnp.exp(t)) + 1e-6
        pq, pk = phi(q), phi(k)
        kv = jnp.einsum("bhsd,bhse->bhde", pk, v)
        z = jnp.einsum("bhsd->bhd", pk)
        num = jnp.einsum("bhqd,bhde->bhqe", pq, kv)
        den = jnp.einsum("bhqd,bhd->bhq", pq, z)[..., None] + 1e-6
        o = num / den
        return (lambda x, *d: x.transpose(*d))(o, 0, 2, 1, 3).reshape(B, S, D) @ wo

    a = _A_ref(A_x, A_wqkv, A_wo)
    b = _B_ref(B_x, B_wqkv, B_wo)
    return jnp.concatenate([a, b], axis=-1)
```

```python
import jax
import jax.numpy as jnp
from jax import lax
import jax.experimental.pallas as pl
import jax.experimental.pallas.tpu as pltpu

S, D, H, DH, NT, W, DIL = 2048, 640, 32, 20, 5, 8, 2
LOG2E = 1.4426950408889634
TM = 256
NB = S // TM
HALO = 16
R = 16
NG = TM // R
F32 = jnp.float32
BF16 = jnp.bfloat16
U32 = jnp.uint32
KV_RANGES = ((0, 144), (112, 272), (240, 400), (368, 528), (496, 640))
PROFILE = False


def _dot(a, b):
    return jnp.dot(a, b, preferred_element_type=F32)


def _dot_nt(a, b):
    return lax.dot_general(a, b, (((1,), (1,)), ((), ())), preferred_element_type=F32)


def _as_bf16(x):
    return pltpu.bitcast(x, BF16)


def _as_u32(x):
    return pltpu.bitcast(x, U32)


def _tile(c, base=0):
    return slice(base + 128 * c, base + 128 * (c + 1))


def _phi(t):
    return jnp.where(t > 0, t + (1.0 + 1e-6), jnp.exp(t) + 1e-6)


def _recip(d):
    r = pl.reciprocal(d, approx=True)
    return r * (2.0 - d * r)


def _lane_allreduce(p):
    p = p + pltpu.roll(p, 64, 1)
    return p + pltpu.roll(p, 32, 1)


def _perm_tables():
    lane = lax.broadcasted_iota(jnp.int32, (8, 128), 1)
    a = (lane >> 2) % 5
    bits = [(a & (1 << s)) != 0 for s in range(3)]
    idx = [(20 * (lane & 31) + 4 * j + (lane >> 5)) & 127 for j in range(NT)]
    return bits, idx


def _permute_cols(tiles, tables):
    bits, idx = tables
    u = [tiles[(3 * p) % 5] for p in range(NT)]
    for s in range(3):
        u = [jnp.where(bits[s], u[(p - (1 << s)) % 5], u[p]) for p in range(NT)]
    return [jnp.take_along_axis(u[j], idx[j], axis=1) for j in range(NT)]


def _permute_weight_cols(src_ref, src_col, dst_ref, dst_col):
    tables = _perm_tables()
    for r in range(0, D // 2, 8):
        tiles = [_as_u32(src_ref[2 * r:2 * r + 16, _tile(i, src_col)]) for i in range(NT)]
        res = _permute_cols(tiles, tables)
        for j in range(NT):
            dst_ref[r:r + 8, _tile(j, dst_col)] = res[j]


def _permute_rows(tmp_ref, dst_ref):
    for c in range(NT):
        for d in range(DH):
            blk = tmp_ref[c, pl.ds(d, H, stride=DH), :]
            dst_ref[16 * d:16 * (d + 1), _tile(c)] = _as_u32(blk.astype(BF16))


def _or_all(vals):
    while len(vals) > 1:
        vals = [vals[i] | vals[i + 1] if i + 1 < len(vals) else vals[i] for i in range(0, len(vals), 2)]
    return vals[0]


def _kernel(ax_hbm, awqkv_hbm, awo_hbm, bx_hbm, bwqkv_hbm, bwo_hbm, out_hbm,
            ax, bx, awqkv, awo, bwqkv, bwo,
            awp, awop, bwqp, mp, wkt, tmpa, tmpb, tmpz,
            q_s, k_s, v_s, o_s, g_acc, zp, pqn_s,
            outa, outb, sem_in, sem_out):

    def rows(b, n=1):
        return slice(b * TM, (b + n) * TM)

    def hrows(b, n=1):
        return slice(b * TM // 2, (b + n) * TM // 2)

    n_in = [0]

    def cp_in(src, dst):
        c = pltpu.make_async_copy(src, dst, sem_in.at[n_in[0]])
        n_in[0] += 1
        return c

    def cp_x(hbm, vm, b, n):
        return cp_in(hbm.at[rows(b, n), :], vm.at[rows(b, n), :])

    def cp_wcols(hbm, vm, c0, c1):
        return cp_in(hbm.at[:, c0:c1], vm.at[:, c0:c1])

    outs = []

    def start_out(src, r, col0):
        c = pltpu.make_async_copy(src.at[r, :], out_hbm.at[r, col0:col0 + D], sem_out.at[len(outs)])
        outs.append(c)
        c.start()

    state = {"z": None, "pkt": {}, "pq": {}, "deps": []}
    scale = DH ** -0.5 * LOG2E

    def wait(name, *cps):
        def go():
            for c in cps:
                c.wait()
        if PROFILE:
            with jax.named_scope(name):
                go()
        else:
            go()

    def b_k(t):
        kt = _dot_nt(_as_bf16(wkt[...]), bx[128 * t:128 * (t + 1), :])
        pk = _phi(kt)
        state["z"] = pk if state["z"] is None else state["z"] + pk
        state["pkt"][t] = pk.astype(BF16)

    def b_g(p):
        pkt = jnp.concatenate([state["pkt"].pop(4 * p + t) for t in range(4)], axis=1)
        g = _dot(pkt, bx[rows(2 * p, 2), :])
        if p == 0:
            g_acc[...] = g
        else:
            g_acc[...] += g

    def a_proj(i, sec):
        y = _dot(ax[rows(i), :], _as_bf16(awp[:, sec * D:(sec + 1) * D]))
        dst, off = ((q_s, 0), (k_s, HALO), (v_s, HALO))[sec]
        for c in range(NT):
            dst[c, off + i * TM: off + (i + 1) * TM, :] = y[:, _tile(c)]

    def a_attn(i, g):
        r0 = i * TM + g * R
        sc = jnp.full((8, 128), scale, F32)
        if state["deps"]:
            always = k_s[0, 0:8, :] == 0.0
            sc = jnp.where(always, sc, pltpu.bitcast(_or_all(state["deps"]), F32))
            state["deps"] = []
        sc = jnp.concatenate([sc] * (R // 8), axis=0)
        q = [q_s[c, r0:r0 + R, :] * sc for c in range(NT)]
        ls = []
        for w in range(W):
            st = HALO + r0 - DIL * w
            p = q[0] * k_s[0, st:st + R, :]
            for c in range(1, NT):
                p = p + q[c] * k_s[c, st:st + R, :]
            p = _lane_allreduce(p)
            if r0 == 0 and w > 0:
                pos = lax.broadcasted_iota(jnp.int32, (R, 128), 0)
                p = jnp.where(pos >= DIL * w, p, -1e9 * LOG2E)
            ls.append(p)
        m = ls[0]
        for w in range(1, W):
            m = jnp.maximum(m, ls[w])
        es = [jnp.exp2(l - m) for l in ls]
        den = es[0]
        for w in range(1, W):
            den = den + es[w]
        inv = _recip(den)
        for c in range(NT):
            st = HALO + r0
            acc = es[0] * v_s[c, st:st + R, :]
            for w in range(1, W):
                st = HALO + r0 - DIL * w
                acc = acc + es[w] * v_s[c, st:st + R, :]
            o = _as_u32((acc * inv).astype(BF16))
            o_s[r0 // 2:(r0 + R) // 2, _tile(c)] = o
            state["deps"].append(o)

    def a_out(i):
        outa[rows(i), :] = _dot(_as_bf16(o_s[hrows(i), :]), _as_bf16(awop[...])).astype(BF16)
        start_out(outa, rows(i), 0)

    def b_q(b, c):
        state["pq"][c] = _phi(_dot(bx[rows(b), :], _as_bf16(bwqp[:, _tile(c)])))

    def b_norm(b):
        pq = [state["pq"].pop(c) for c in range(NT)]
        t = pq[0] * zp[0:1, _tile(0)]
        for c in range(1, NT):
            t = t + pq[c] * zp[0:1, _tile(c)]
        inv = _recip(_lane_allreduce(t) + 1e-6)
        for c in range(NT):
            pqn_s[hrows(b), _tile(c)] = _as_u32((pq[c] * inv).astype(BF16))
        iu = _as_u32(inv)
        state["deps"] += [iu[8 * j:8 * (j + 1), :] for j in range(TM // 8)]

    def b_out(b):
        outb[rows(b), :] = _dot(_as_bf16(pqn_s[hrows(b), :]), _as_bf16(mp[...])).astype(BF16)
        start_out(outb, rows(b), D)

    def b_fin_z():
        tmpz[...] = state["z"]
        for j in range(NT):
            zr = jnp.concatenate([tmpz[pl.ds(4 * j + dl, H, stride=DH), :] for dl in range(4)], axis=0)
            zr = jnp.sum(zr.T, axis=0, keepdims=True)
            zp[:, _tile(j)] = jnp.broadcast_to(zr, (8, 128))

    def b_fin_m():
        kvs = []
        for j, (lo, hi) in enumerate(KV_RANGES):
            kv = _dot(g_acc[lo:hi, :].astype(BF16), bwqkv[:, _tile(j, 2 * D)])
            rh = (lax.broadcasted_iota(jnp.int32, (hi - lo, 128), 0) + lo) // DH
            ch = (lax.broadcasted_iota(jnp.int32, (hi - lo, 128), 1) + 128 * j) // DH
            kvs.append(jnp.where(rh == ch, kv, 0.0).astype(BF16))
        prev_hi = 0
        for j, (lo, hi) in enumerate(KV_RANGES):
            mj = _dot(kvs[j], bwo[_tile(j), :])
            ov = prev_hi - lo
            for c in range(NT):
                if ov > 0:
                    tmpb[c, lo:prev_hi, :] += mj[0:ov, _tile(c)]
                tmpb[c, lo + max(ov, 0):hi, :] = mj[max(ov, 0):, _tile(c)]
            prev_hi = hi
        _permute_rows(tmpb, mp)

    def perm_awo():
        for c in range(NT):
            tmpa[c] = awo[:, _tile(c)].astype(F32)
        _permute_rows(tmpa, awop)

    d_bwk = cp_wcols(bwqkv_hbm, bwqkv, D, 2 * D)
    d_bx0 = cp_x(bx_hbm, bx, 0, 2)
    d_bxr = cp_x(bx_hbm, bx, 2, NB - 2)
    d_aw = cp_in(awqkv_hbm, awqkv)
    d_bwq = cp_wcols(bwqkv_hbm, bwqkv, 0, D)
    d_awo = cp_in(awo_hbm, awo)
    d_bwv = cp_wcols(bwqkv_hbm, bwqkv, 2 * D, 3 * D)
    d_bwo = cp_in(bwo_hbm, bwo)
    d_ax = cp_in(ax_hbm, ax)

    d_bwk.start()
    d_bx0.start()
    for c in range(NT):
        k_s[c, 0:HALO, :] = jnp.zeros((HALO, 128), F32)
        v_s[c, 0:HALO, :] = jnp.zeros((HALO, 128), F32)
    wait("w0a", d_bwk)
    d_bxr.start()
    wkt[...] = _as_u32(bwqkv[:, D:2 * D].T)
    wait("w0b", d_bx0)
    for d in (d_aw, d_bwq, d_awo, d_bwv, d_bwo, d_ax):
        d.start()
    for t in range(4):
        b_k(t)
    b_g(0)
    wait("w1", d_bxr)
    for p in range(1, 4):
        for t in range(4):
            b_k(4 * p + t)
        if p < 3:
            b_g(p)
    wait("w2", d_aw, d_bwq, d_awo, d_bwv, d_bwo, d_ax)
    b_g(3)
    for sec in (2, 1, 0):
        _permute_weight_cols(awqkv, sec * D, awp, sec * D)
    _permute_weight_cols(bwqkv, 0, bwqp, 0)
    b_fin_z()
    perm_awo()

    for i in range(NB):
        a_proj(i, 2)
        a_proj(i, 1)
        a_proj(i, 0)
        if i == 0:
            b_fin_m()
        for g in range(NG):
            a_attn(i, g)
            if g < NT:
                b_q(i, g)
            if g == NT - 1:
                b_norm(i)
                if i >= 2:
                    b_out(i - 2)
                if i >= 1:
                    a_out(i - 1)
                if i == NB - 1:
                    b_out(NB - 2)
                    b_out(NB - 1)
    a_out(NB - 1)

    wait("wend", *outs)


@jax.jit
def pallas_concat_heads__sliding_local_dilated__linear_attn_block__prompt_kernel(
    A_x, A_wqkv, A_wo, B_x, B_wqkv, B_wo,
):
    any_spec = pl.BlockSpec(memory_space=pl.ANY)
    out = pl.pallas_call(
        _kernel,
        in_specs=[any_spec] * 6,
        out_specs=any_spec,
        out_shape=jax.ShapeDtypeStruct((S, 2 * D), BF16),
        scratch_shapes=[
            pltpu.VMEM((S, D), BF16), pltpu.VMEM((S, D), BF16),
            pltpu.VMEM((D, 3 * D), BF16), pltpu.VMEM((D, D), BF16),
            pltpu.VMEM((D, 3 * D), BF16), pltpu.VMEM((D, D), BF16),
            pltpu.VMEM((D // 2, 3 * D), U32), pltpu.VMEM((D // 2, D), U32),
            pltpu.VMEM((D // 2, D), U32), pltpu.VMEM((D // 2, D), U32), pltpu.VMEM((D // 2, D), U32),
            pltpu.VMEM((NT, D, 128), F32), pltpu.VMEM((NT, D, 128), F32), pltpu.VMEM((D, 128), F32),
            pltpu.VMEM((NT, S, 128), F32), pltpu.VMEM((NT, S + HALO, 128), F32),
            pltpu.VMEM((NT, S + HALO, 128), F32), pltpu.VMEM((S // 2, D), U32),
            pltpu.VMEM((D, D), F32), pltpu.VMEM((8, D), F32), pltpu.VMEM((S // 2, D), U32),
            pltpu.VMEM((S, D), BF16), pltpu.VMEM((S, D), BF16),
            pltpu.SemaphoreType.DMA((16,)), pltpu.SemaphoreType.DMA((16,)),
        ],
        compiler_params=pltpu.CompilerParams(vmem_limit_bytes=100 * 2**20),
        name="fused_ab",
    )(A_x.reshape(S, D), A_wqkv, A_wo, B_x.reshape(S, D), B_wqkv, B_wo)
    return out.reshape(1, S, 2 * D)
```

```python
import jax
import jax.numpy as jnp
from jax import lax
import jax.experimental.pallas as pl
import jax.experimental.pallas.tpu as pltpu

S, D, H, DH, NT, W, DIL = 2048, 640, 32, 20, 5, 8, 2
LOG2E = 1.4426950408889634
TM = 256
NB = S // TM
HALO = 16
NG = TM // 8
F32 = jnp.float32
BF16 = jnp.bfloat16
U32 = jnp.uint32
KV_RANGES = ((0, 144), (120, 264), (240, 400), (376, 520), (496, 640))
PERM_DEPTH = 5
G3_SPLIT = 2
GATE_W = 4


def _dot(a, b):
    return jnp.dot(a, b, preferred_element_type=F32)


def _dot_nt(a, b):
    return lax.dot_general(a, b, (((1,), (1,)), ((), ())), preferred_element_type=F32)


def _tile(c, base=0):
    return slice(base + 128 * c, base + 128 * (c + 1))


def _bf16(x):
    return pltpu.bitcast(x, BF16)


def _u32(x):
    return pltpu.bitcast(x, U32)


def _f32(x):
    return pltpu.bitcast(x, F32)


def _phi(t, log2e=LOG2E):
    return jnp.where(t > 0, t + (1.0 + 1e-6), jnp.exp2(t * log2e) + 1e-6)


def _recip(d):
    r = pl.reciprocal(d, approx=True)
    return r * (2.0 - d * r)


def _head_sum(p):
    r = [pltpu.roll(p, 32 * k, 1) for k in (1, 2, 3)]
    return (p + r[0]) + (r[1] + r[2]), r


def _perm_tables():
    lane = lax.broadcasted_iota(jnp.int32, (8 * NT, 128), 1)
    j = lax.broadcasted_iota(jnp.int32, (8 * NT, 128), 0) >> 3
    a = (lane >> 2) % 5
    idx = (20 * (lane & 31) + 4 * j + (lane >> 5)) & 127
    return a & 1, (a & 2) != 0, (a & 4) != 0, idx


def _permute_cols(x, tables, zero):
    a1, bit2, bit4, idx = tables
    u = jnp.concatenate([x[:, _tile((3 * p) % 5)] for p in range(NT)], axis=0)
    for mask, k in ((a1 != jnp.concatenate([zero] * NT, axis=0), 1), (bit2, 2), (bit4, 4)):
        u = jnp.where(mask, jnp.concatenate([u[8 * (NT - k):], u[:8 * (NT - k)]], axis=0), u)
    u = jnp.take_along_axis(u, idx, axis=1, mode="promise_in_bounds")
    return jnp.concatenate([u[8 * j:8 * (j + 1)] for j in range(NT)], axis=1)


def _tree_max(vals):
    while len(vals) > 1:
        vals = [jnp.maximum(vals[i], vals[i + 1]) if i + 1 < len(vals) else vals[i]
                for i in range(0, len(vals), 2)]
    return vals[0]


def _halve(op, x):
    while x.shape[0] > 1:
        n = x.shape[0] // 2
        x = op(x[:n], x[n:])
    return x


def _fold(x):
    if x.ndim == 2:
        x = jnp.concatenate([x[:, _tile(c)] for c in range(x.shape[1] // 128)], axis=0)
        x = x.reshape(x.shape[0] // 8, 8, 128)
    return jnp.max(x, axis=0)


def _kernel(ax_hbm, awqkv_hbm, awo_hbm, bx_hbm, bwqkv_hbm, bwo_hbm, out_hbm,
            ax, bx, awqkv, awo, bwqkv, bwo,
            awp, awo_u, awop, bwqp, mp, wkt, tmpb, tmpz,
            q_s, k_s, v_s, o_s, g_acc, zp, qb_s, pqn_s, pkt_s,
            outa, outb, sems):

    def rows(b, n=1):
        return slice(b * TM, (b + n) * TM)

    def lanes(ref, r):
        return jnp.concatenate([ref[c, r, :] for c in range(NT)], axis=1)

    def cp_rows(hbm, vm, r, sem):
        return pltpu.make_async_copy(hbm.at[r, :], vm.at[r, :], sems.at[sem])

    def cp_cols(hbm, vm, c0, c1, sem):
        return pltpu.make_async_copy(hbm.at[:, c0:c1], vm.at[:, c0:c1], sems.at[sem])

    outs = []

    def start_out(src, r, col0):
        c = pltpu.make_async_copy(src.at[r, :], out_hbm.at[r, col0:col0 + D], sems.at[4])
        outs.append(c)
        c.start()

    state = {"z": None, "z0": {}, "perm": [], "k0": {}, "deps": [[], []], "half": {}}

    def wait(*cps):
        for c in cps:
            c.wait()

    def gated(consts, deps):
        vals = [jnp.full((8, 128), c, F32) for c in consts]
        if not deps:
            return vals
        always = k_s[0, 0:8, :] == 0.0
        dep = _tree_max(deps)
        return [jnp.where(always, v, dep) for v in vals]

    def gate_rhs(rhs, gates):
        if not gates:
            return rhs
        nk, nn = rhs.shape[0] // 128, rhs.shape[1] // 128
        always = k_s[0, 0:8, :] == 0.0
        cols = []
        for n in range(nn):
            parts = []
            for k in range(nk):
                tile = rhs[_tile(k), _tile(n)]
                dep = gates.get(n * nk + k)
                if dep is not None:
                    tail = _bf16(jnp.where(always, _f32(tile[112:, :]), dep))
                    tile = jnp.concatenate([tile[:112, :], tail], axis=0)
                parts.append(tile)
            cols.append(jnp.concatenate(parts, axis=0))
        return jnp.concatenate(cols, axis=1)

    def permute_weight_cols(tables, src_ref, src_col, dst_ref, dst_col):
        chain = state["perm"]
        for r in range(0, D, 16):
            after = [chain[-PERM_DEPTH]] if len(chain) >= PERM_DEPTH else []
            zero = pltpu.bitcast(gated((0.0,), after)[0], jnp.int32)
            res = _permute_cols(_u32(src_ref[r:r + 16, src_col:src_col + D]), tables, zero)
            dst_ref[r // 2:r // 2 + 8, dst_col:dst_col + D] = res
            chain.append(_f32(res[:, _tile(NT - 1)]))
        return _fold(_f32(res))

    def permute_m_rows(d):
        val = jnp.concatenate([tmpb[c, pl.ds(d, H, stride=DH), :] for c in range(NT)], axis=1)
        val = _u32(val.astype(BF16))
        mp[16 * d:16 * (d + 1), :] = val
        return _fold(_f32(val))

    def repack_wo(c):
        val = _u32(awo[:, _tile(c)])
        awo_u[c] = val
        return _fold(_f32(val))

    def permute_wo_rows(dp):
        a = jnp.concatenate([awo_u[c, pl.ds(dp, 16, stride=DH), :] for c in range(NT)], axis=1)
        b = jnp.concatenate([awo_u[c, pl.ds(dp + DH // 2, 16, stride=DH), :] for c in range(NT)], axis=1)
        val = jnp.concatenate([(a & 0xFFFF) | (b << 16), (a >> 16) | (b & jnp.uint32(0xFFFF0000))], axis=0)
        awop[32 * dp:32 * (dp + 1), :] = val
        return _fold(_f32(val))

    def b_k_first_dot(c, m):
        state["k0"][c] = jnp.concatenate(
            [_dot(bx[r:r + m, :], bwqkv[:, _tile(c, D)]) for r in range(0, 2 * TM, m)], axis=0)

    def b_k_first(c):
        pk = _phi(state["k0"].pop(c))
        state["z0"][c] = jnp.sum(pk.reshape(2 * TM // 8, 8, 128), axis=0)
        pkt_s[64 * c:64 * (c + 1), rows(0, 2)] = _u32(pk.astype(BF16).T)

    def b_k(t):
        pk = _phi(_dot_nt(_bf16(wkt[...]), bx[_tile(t), :]))
        state["z"] = pk if state["z"] is None else state["z"] + pk
        pkt_s[:, _tile(t)] = _u32(pk.astype(BF16))

    def b_g(p, gates=None, c0=0, c1=NT):
        cols = slice(128 * c0, 128 * c1)
        g = _dot(_bf16(pkt_s[:, rows(2 * p, 2)]), gate_rhs(bx[rows(2 * p, 2), cols], gates))
        if p == 0:
            g_acc[:, cols] = g
        else:
            g_acc[:, cols] += g

    def b_fin_z(tables):
        tmpz[...] = state["z"]
        z0 = jnp.concatenate([state["z0"][c] for c in range(NT)], axis=1)
        z0 = _permute_cols(z0, tables, jnp.zeros((8, 128), jnp.int32))
        for j in range(NT):
            zr = jnp.concatenate([tmpz[pl.ds(4 * j + dl, H, stride=DH), :] for dl in range(4)], axis=0)
            zr = jnp.sum(zr.T, axis=0, keepdims=True) + jnp.sum(z0[:, _tile(j)], axis=0, keepdims=True)
            zp[j] = jnp.broadcast_to(zr, (8, 128))

    def b_fin_kv():
        kvs = state["kv"] = []
        for j, (lo, hi) in enumerate(KV_RANGES):
            kv = _dot(g_acc[lo:hi, :].astype(BF16), bwqkv[:, _tile(j, 2 * D)])
            head0 = ((lax.broadcasted_iota(jnp.int32, (1, 128), 1) + 128 * j) // DH) * DH - lo
            rel = lax.broadcasted_iota(jnp.int32, (hi - lo, 128), 0) - head0
            kvs.append(jnp.where((rel >= 0) & (rel < DH), kv, 0.0).astype(BF16))

    def b_fin_m():
        prev_hi = 0
        for j, (lo, hi) in enumerate(KV_RANGES):
            mj = _dot(state["kv"][j], bwo[_tile(j), :])
            ov = max(prev_hi - lo, 0)
            for c in range(NT):
                if ov:
                    tmpb[c, lo:prev_hi, :] += mj[0:ov, _tile(c)]
                tmpb[c, lo + ov:hi, :] = mj[ov:, _tile(c)]
            prev_hi = hi

    def a_proj(i, sec, gates=None):
        y = _dot(ax[rows(i), :], gate_rhs(_bf16(awp[:, sec * D:(sec + 1) * D]), gates))
        dst, off = ((q_s, 0), (k_s, HALO), (v_s, HALO))[sec]
        for c in range(NT):
            dst[c, off + i * TM: off + (i + 1) * TM, :] = y[:, _tile(c)]

    def b_q(b):
        y = _dot(bx[rows(b), :], _bf16(bwqp[...]))
        for c in range(NT):
            qb_s[c, rows(b), :] = y[:, _tile(c)]

    def a_out(r):
        outa[r, :] = _dot(lanes(o_s, r), _bf16(awop[...])).astype(BF16)
        start_out(outa, r, 0)

    def b_out(r):
        outb[r, :] = _dot(lanes(pqn_s, r), _bf16(mp[...])).astype(BF16)
        start_out(outb, r, D)

    def store_pair(key, dst, r0, val):
        if r0 % 16 == 0:
            state["half"][key] = val
        else:
            dst[:, r0 - 8:r0 + 8, :] = jnp.concatenate([state["half"].pop(key), val], axis=1).astype(BF16)

    def group(i, g):
        r0 = i * TM + g * 8
        sc, l2e = gated((DH ** -0.5 * LOG2E, LOG2E), state["deps"][g % 2])
        deps = state["deps"][g % 2] = []

        q = q_s[:, r0:r0 + 8, :] * sc[None]
        ls = []
        for w in range(W):
            st = HALO + r0 - DIL * w
            p, r = _head_sum(jnp.sum(q * k_s[:, st:st + 8, :], axis=0))
            if w == GATE_W:
                state["deps"][(g + 1) % 2].extend(r[:2])
            if r0 < DIL * w:
                pos = lax.broadcasted_iota(jnp.int32, (8, 128), 0) + r0
                p = jnp.where(pos >= DIL * w, p, -1e9 * LOG2E)
            ls.append(p)

        pq = _phi(qb_s[:, r0:r0 + 8, :], l2e[None])
        den, _ = _head_sum(jnp.sum(pq * zp[...], axis=0))

        ls = jnp.stack(ls)
        es = jnp.exp2(ls - _halve(jnp.maximum, ls))
        inv = _recip(_halve(jnp.add, es))
        acc = es[0:1] * v_s[:, HALO + r0:HALO + r0 + 8, :]
        for w in range(1, W):
            st = HALO + r0 - DIL * w
            acc = acc + es[w:w + 1] * v_s[:, st:st + 8, :]
        o = acc * inv
        store_pair("o", o_s, r0, o)

        pqn = pq * _recip(den + 1e-6)[None]
        store_pair("pqn", pqn_s, r0, pqn)
        deps.append(_fold(jnp.maximum(o, pqn)))

    d_bx0 = cp_rows(bx_hbm, bx, rows(0, 2), 0)
    d_bwk = [cp_cols(bwqkv_hbm, bwqkv, D + c0, D + c1, sem)
             for c0, c1, sem in ((0, 128, 0), (128, 256, 1), (256, 384, 2), (384, D, 5))]
    d_bxr = cp_rows(bx_hbm, bx, rows(2, NB - 2), 0)
    d_rest = [
        cp_cols(bwqkv_hbm, bwqkv, 0, D, 3),
        pltpu.make_async_copy(awqkv_hbm, awqkv, sems.at[3]),
        pltpu.make_async_copy(awo_hbm, awo, sems.at[3]),
        cp_cols(bwqkv_hbm, bwqkv, 2 * D, 3 * D, 3),
        pltpu.make_async_copy(bwo_hbm, bwo, sems.at[3]),
        pltpu.make_async_copy(ax_hbm, ax, sems.at[3]),
    ]

    d_bx0.start()
    for d in d_bwk:
        d.start()
    k_s[:, 0:HALO, :] = jnp.zeros((NT, HALO, 128), F32)
    v_s[:, 0:HALO, :] = jnp.zeros((NT, HALO, 128), F32)
    wait(d_bx0, d_bwk[0])
    d_bxr.start()
    b_k_first_dot(0, 128)
    wait(d_bwk[1])
    b_k_first_dot(1, 128)
    wait(d_bwk[2])
    for d in d_rest:
        d.start()
    b_k_first_dot(2, 128)
    b_k_first(0)
    wait(d_bwk[3])
    b_k_first_dot(3, 256)
    b_k_first_dot(4, 256)
    for c in range(1, NT):
        b_k_first(c)
    wkt[...] = _u32(bwqkv[:, D:2 * D].T)
    b_g(0, {8: _fold(_f32(wkt[D // 2 - 8:, :]))})
    wait(d_bxr)
    for p in range(1, 4):
        for t in range(4):
            b_k(4 * p + t)
        if p == 3:
            b_fin_z(_perm_tables())
        b_g(p, None, 0, NT if p < 3 else G3_SPLIT)
    wait(*d_rest)
    tables = _perm_tables()
    permute_weight_cols(tables, bwqkv, 0, bwqp, 0)
    for sec in (2, 1, 0):
        dep_q = permute_weight_cols(tables, awqkv, sec * D, awp, sec * D)
    b_g(3, None, G3_SPLIT, NT)
    b_q(0)

    for i in range(NB):
        if i == 0:
            a_proj(0, 2, {24: dep_q, **{3 + 4 * c: repack_wo(c) for c in range(NT)}})
            b_fin_kv()
            a_proj(0, 1, {4 + 2 * dp: permute_wo_rows(dp) for dp in range(DH // 2)})
            b_fin_m()
            a_proj(0, 0)
        else:
            a_proj(i, 2)
            a_proj(i, 1)
            a_proj(i, 0, {4 + d: permute_m_rows(d) for d in range(DH)} if i == 1 else None)
        if i + 1 < NB:
            b_q(i + 1)
        for g in range(NG):
            group(i, g)
        if i >= 2:
            b_out(rows(i - 2))
        if i >= 1:
            a_out(rows(i - 1))
    b_out(rows(NB - 2))
    b_out(rows(NB - 1))
    a_out(slice(S - TM, S - 128))
    a_out(slice(S - 128, S - 64))
    a_out(slice(S - 64, S))

    wait(*outs)


@jax.jit
def pallas_concat_heads__sliding_local_dilated__linear_attn_block__prompt_kernel(
    A_x, A_wqkv, A_wo, B_x, B_wqkv, B_wo,
):
    def bf(*shape):
        return pltpu.VMEM(shape, BF16)

    def f32(*shape):
        return pltpu.VMEM(shape, F32)

    def packed(r, c):
        return pltpu.VMEM((r // 2, c), U32)

    any_spec = pl.BlockSpec(memory_space=pl.ANY)
    out = pl.pallas_call(
        _kernel,
        in_specs=[any_spec] * 6,
        out_specs=any_spec,
        out_shape=jax.ShapeDtypeStruct((S, 2 * D), BF16),
        scratch_shapes=[
            bf(S, D), bf(S, D), bf(D, 3 * D), bf(D, D), bf(D, 3 * D), bf(D, D),
            packed(D, 3 * D), pltpu.VMEM((NT, D // 2, 128), U32), packed(D, D), packed(D, D), packed(D, D),
            packed(D, D), f32(NT, D, 128), f32(D, 128),
            f32(NT, S, 128), f32(NT, S + HALO, 128), f32(NT, S + HALO, 128), bf(NT, S, 128),
            f32(D, D), f32(NT, 8, 128), f32(NT, S, 128), bf(NT, S, 128), packed(D, S),
            bf(S, D), bf(S, D),
            pltpu.SemaphoreType.DMA((6,)),
        ],
        compiler_params=pltpu.CompilerParams(vmem_limit_bytes=100 * 2**20),
        name="fused_ab",
    )(A_x.reshape(S, D), A_wqkv, A_wo, B_x.reshape(S, D), B_wqkv, B_wo)
    return out.reshape(1, S, 2 * D)
```

```python
import jax
import jax.numpy as jnp
from jax import lax
import jax.experimental.pallas as pl
import jax.experimental.pallas.tpu as pltpu

S, D, H, DH, NT, W, DIL = 2048, 640, 32, 20, 5, 8, 2
LOG2E = 1.4426950408889634
TM = 256
NB = S // TM
PAD = 24
HALO = 16
NG = TM // 8
F32 = jnp.float32
BF16 = jnp.bfloat16
U32 = jnp.uint32
KV_RANGES = ((0, 144), (120, 264), (240, 400), (376, 520), (496, 640))
NF = 4
PERM_DEPTH = 5
G3_SPLIT = 3
GATE_W = 4


def _dot(a, b):
    return jnp.dot(a, b, preferred_element_type=F32)


def _dot_nt(a, b):
    return lax.dot_general(a, b, (((1,), (1,)), ((), ())), preferred_element_type=F32)


def _tile(c, base=0):
    return slice(base + 128 * c, base + 128 * (c + 1))


def _bf16(x):
    return pltpu.bitcast(x, BF16)


def _u32(x):
    return pltpu.bitcast(x, U32)


def _f32(x):
    return pltpu.bitcast(x, F32)


def _phi(t, log2e=LOG2E):
    return jnp.where(t > 0, t + (1.0 + 1e-6), jnp.exp2(t * log2e) + 1e-6)


def _recip(d):
    r = pl.reciprocal(d, approx=True)
    return r * (2.0 - d * r)


def _head_sum(p):
    r = [pltpu.roll(p, 32 * k, 1) for k in (1, 2, 3)]
    return (p + r[0]) + (r[1] + r[2]), r


def _perm_tables():
    lane = lax.broadcasted_iota(jnp.int32, (8 * NT, 128), 1)
    j = lax.broadcasted_iota(jnp.int32, (8 * NT, 128), 0) >> 3
    a = (lane >> 2) % 5
    idx = (20 * (lane & 31) + 4 * j + (lane >> 5)) & 127
    return a & 1, (a & 2) != 0, (a & 4) != 0, idx


def _permute_cols(x, tables, zero):
    a1, bit2, bit4, idx = tables
    u = jnp.concatenate([x[:, _tile((3 * p) % 5)] for p in range(NT)], axis=0)
    for mask, k in ((a1 != jnp.concatenate([zero] * NT, axis=0), 1), (bit2, 2), (bit4, 4)):
        u = jnp.where(mask, jnp.concatenate([u[8 * (NT - k):], u[:8 * (NT - k)]], axis=0), u)
    u = jnp.take_along_axis(u, idx, axis=1, mode="promise_in_bounds")
    return jnp.concatenate([u[8 * j:8 * (j + 1)] for j in range(NT)], axis=1)


def _tree_max(vals):
    while len(vals) > 1:
        vals = [jnp.maximum(vals[i], vals[i + 1]) if i + 1 < len(vals) else vals[i]
                for i in range(0, len(vals), 2)]
    return vals[0]


def _halve(op, x):
    while x.shape[0] > 1:
        n = x.shape[0] // 2
        x = op(x[:n], x[n:])
    return x


def _fold(x):
    if x.ndim == 2:
        x = jnp.concatenate([x[:, _tile(c)] for c in range(x.shape[1] // 128)], axis=0)
        x = x.reshape(x.shape[0] // 8, 8, 128)
    return jnp.max(x, axis=0)


def _kernel(ax_hbm, awqkv_hbm, awo_hbm, bx_hbm, bwqkv_hbm, bwo_hbm, out_hbm,
            ax, bx, awqkv, awo, bwqkv, bwo,
            awp, awo_u, awop, bwqp, mp, wkt, tmpb, tmpz,
            q_s, k_s, v_s, o_s, g_acc, zp, qb_s, pqn_s, pkt_s,
            outa, outb, sems):

    def rows(b, n=1):
        return slice(b * TM, (b + n) * TM)

    def lanes(ref, r):
        return jnp.concatenate([ref[c, r, :] for c in range(NT)], axis=1)

    def cp_rows(hbm, vm, r, sem):
        return pltpu.make_async_copy(hbm.at[r, :], vm.at[r, :], sems.at[sem])

    def cp_cols(hbm, vm, c0, c1, sem):
        return pltpu.make_async_copy(hbm.at[:, c0:c1], vm.at[:, c0:c1], sems.at[sem])

    outs = []

    def start_out(src, r, col0):
        c = pltpu.make_async_copy(src.at[r, :], out_hbm.at[r, col0:col0 + D], sems.at[4])
        outs.append(c)
        c.start()

    state = {"z": None, "perm": [], "k0": {}, "deps": [[], []], "half": {}}

    def wait(*cps):
        for c in cps:
            c.wait()

    def gated(consts, deps):
        vals = [jnp.full((8, 128), c, F32) for c in consts]
        if not deps:
            return vals
        always = k_s[0, 0:8, :] == 0.0
        dep = _tree_max(deps)
        return [jnp.where(always, v, dep) for v in vals]

    def gate_rhs(rhs, gates):
        if not gates:
            return rhs
        nk, nn = rhs.shape[0] // 128, rhs.shape[1] // 128
        always = k_s[0, 0:8, :] == 0.0
        cols = []
        for n in range(nn):
            parts = []
            for k in range(nk):
                tile = rhs[_tile(k), _tile(n)]
                dep = gates.get(n * nk + k)
                if dep is not None:
                    tail = _bf16(jnp.where(always, _u32(tile[112:, :]), _u32(dep)))
                    tile = jnp.concatenate([tile[:112, :], tail], axis=0)
                parts.append(tile)
            cols.append(jnp.concatenate(parts, axis=0))
        return jnp.concatenate(cols, axis=1)

    def permute_weight_cols(tables, src_ref, src_col, dst_ref, dst_col):
        chain = state["perm"]
        for r in range(0, D, 16):
            after = [chain[-PERM_DEPTH]] if len(chain) >= PERM_DEPTH else []
            zero = pltpu.bitcast(gated((0.0,), after)[0], jnp.int32)
            res = _permute_cols(_u32(src_ref[r:r + 16, src_col:src_col + D]), tables, zero)
            dst_ref[r // 2:r // 2 + 8, dst_col:dst_col + D] = res
            chain.append(_f32(res[:, _tile(NT - 1)]))
        return _fold(_f32(res))

    def permute_m_rows(d):
        val = jnp.concatenate([tmpb[c, pl.ds(d, H, stride=DH), :] for c in range(NT)], axis=1)
        val = _u32(val.astype(BF16))
        mp[16 * d:16 * (d + 1), :] = val
        return _fold(_f32(val))

    def repack_wo(c):
        val = _u32(awo[:, _tile(c)])
        awo_u[c, 0:D // 2, :] = val
        return _fold(_f32(val))

    def permute_wo_rows(dp):
        a = jnp.concatenate([awo_u[c, pl.ds(dp, 16, stride=DH), :] for c in range(NT)], axis=1)
        b = jnp.concatenate([awo_u[c, pl.ds(dp + DH // 2, 16, stride=DH), :] for c in range(NT)], axis=1)
        val = jnp.concatenate([(a & 0xFFFF) | (b << 16), (a >> 16) | (b & jnp.uint32(0xFFFF0000))], axis=0)
        awop[32 * dp:32 * (dp + 1), :] = val
        return _fold(_f32(val))

    def b_k_first(b, c0, c1, m=TM):
        kc = slice(128 * c0, 128 * c1)
        k = jnp.concatenate([_dot(bx[r:r + m, kc], bwqkv[kc, D:2 * D])
                             for r in range(b * TM, (b + 1) * TM, m)], axis=0)
        if c0 > 0:
            k = k + state["k0"].pop(b)
        if c1 < NT:
            state["k0"][b] = k
        else:
            pk = _phi(k)
            z0 = jnp.sum(pk.reshape(TM // 8, 8, D), axis=0)
            state["z0"] = z0 if b == 0 else state["z0"] + z0
            pkt_s[:, rows(b)] = _u32(pk.astype(BF16).T)

    def b_k(t):
        pk = _phi(_dot_nt(_bf16(wkt[...]), bx[_tile(t), :]))
        state["z"] = pk if state["z"] is None else state["z"] + pk
        pkt_s[:, _tile(t)] = _u32(pk.astype(BF16))

    def b_g(p, gates=None, c0=0, c1=NT):
        cols = slice(128 * c0, 128 * c1)
        g = _dot(_bf16(pkt_s[:, rows(2 * p, 2)]), gate_rhs(bx[rows(2 * p, 2), cols], gates))
        if p == 0:
            g_acc[:, cols] = g
        else:
            g_acc[:, cols] += g

    def b_fin_z(tables):
        tmpz[0:D, :] = state["z"]
        z0 = _permute_cols(state["z0"], tables, jnp.zeros((8, 128), jnp.int32))
        for j in range(NT):
            zr = jnp.concatenate([tmpz[pl.ds(4 * j + dl, H, stride=DH), :] for dl in range(4)], axis=0)
            zr = jnp.sum(zr.T, axis=0, keepdims=True) + jnp.sum(z0[:, _tile(j)], axis=0, keepdims=True)
            zp[j] = jnp.broadcast_to(zr, (8, 128))

    def b_fin_kv():
        kvs = state["kv"] = []
        for j, (lo, hi) in enumerate(KV_RANGES):
            kv = _dot(g_acc[lo:hi, :].astype(BF16), bwqkv[:, _tile(j, 2 * D)])
            head0 = ((lax.broadcasted_iota(jnp.int32, (1, 128), 1) + 128 * j) // DH) * DH - lo
            rel = lax.broadcasted_iota(jnp.int32, (hi - lo, 128), 0) - head0
            kvs.append(jnp.where((rel >= 0) & (rel < DH), kv, 0.0).astype(BF16))

    def b_fin_m():
        prev_hi = 0
        for j, (lo, hi) in enumerate(KV_RANGES):
            mj = _dot(state["kv"][j], bwo[_tile(j), :])
            ov = max(prev_hi - lo, 0)
            for c in range(NT):
                if ov:
                    tmpb[c, lo:prev_hi, :] += mj[0:ov, _tile(c)]
                tmpb[c, lo + ov:hi, :] = mj[ov:, _tile(c)]
            prev_hi = hi

    def a_proj(i, sec, gates=None):
        y = _dot(ax[rows(i), :], gate_rhs(_bf16(awp[:, sec * D:(sec + 1) * D]), gates))
        dst, off = ((q_s, 0), (k_s, HALO), (v_s, HALO))[sec]
        for c in range(NT):
            dst[c, off + i * TM: off + (i + 1) * TM, :] = y[:, _tile(c)]

    def b_q(b):
        y = _dot(bx[rows(b), :], _bf16(bwqp[...]))
        for c in range(NT):
            qb_s[c, rows(b), :] = y[:, _tile(c)]

    def a_out(r):
        outa[r, :] = _dot(lanes(o_s, r), _bf16(awop[...])).astype(BF16)
        start_out(outa, r, 0)

    def b_out(r):
        outb[r, :] = _dot(lanes(pqn_s, r), _bf16(mp[...])).astype(BF16)
        start_out(outb, r, D)

    def store_pair(key, dst, r0, val):
        if r0 % 16 == 0:
            state["half"][key] = val
        else:
            dst[:, r0 - 8:r0 + 8, :] = jnp.concatenate([state["half"].pop(key), val], axis=1).astype(BF16)

    def group(i, g):
        r0 = i * TM + g * 8
        sc, l2e = gated((DH ** -0.5 * LOG2E, LOG2E), state["deps"][g % 2])
        deps = state["deps"][g % 2] = []

        q = q_s[:, r0:r0 + 8, :] * sc[None]
        ls = []
        for w in range(W):
            st = HALO + r0 - DIL * w
            p, r = _head_sum(jnp.sum(q * k_s[:, st:st + 8, :], axis=0))
            if w == GATE_W:
                state["deps"][(g + 1) % 2].extend(r[:2])
            if r0 < DIL * w:
                pos = lax.broadcasted_iota(jnp.int32, (8, 128), 0) + r0
                p = jnp.where(pos >= DIL * w, p, -1e9 * LOG2E)
            ls.append(p)

        pq = _phi(qb_s[:, r0:r0 + 8, :], l2e[None])
        den, _ = _head_sum(jnp.sum(pq * zp[...], axis=0))

        ls = jnp.stack(ls)
        es = jnp.exp2(ls - _halve(jnp.maximum, ls))
        inv = _recip(_halve(jnp.add, es))
        acc = es[0:1] * v_s[:, HALO + r0:HALO + r0 + 8, :]
        for w in range(1, W):
            st = HALO + r0 - DIL * w
            acc = acc + es[w:w + 1] * v_s[:, st:st + 8, :]
        o = acc * inv
        store_pair("o", o_s, r0, o)

        pqn = pq * _recip(den + 1e-6)[None]
        store_pair("pqn", pqn_s, r0, pqn)
        deps.append(_fold(jnp.maximum(o, pqn)))

    d_first = [
        (pltpu.make_async_copy(bx_hbm.at[rows(0, NF), _tile(c)], bx.at[rows(0, NF), _tile(c)], sems.at[sem]),
         pltpu.make_async_copy(bwqkv_hbm.at[_tile(c), D:2 * D], bwqkv.at[_tile(c), D:2 * D], sems.at[sem]))
        for c, sem in enumerate((0, 1, 2, 5, 6))]
    d_bxr = cp_rows(bx_hbm, bx, rows(NF, NB - NF), 0)
    d_rest = [
        cp_cols(bwqkv_hbm, bwqkv, 0, D, 3),
        pltpu.make_async_copy(awqkv_hbm, awqkv, sems.at[3]),
        pltpu.make_async_copy(awo_hbm, awo, sems.at[3]),
        cp_cols(bwqkv_hbm, bwqkv, 2 * D, 3 * D, 3),
        pltpu.make_async_copy(bwo_hbm, bwo, sems.at[3]),
        pltpu.make_async_copy(ax_hbm, ax, sems.at[3]),
    ]

    for pair in d_first:
        for d in pair:
            d.start()
    k_s[:, 0:HALO, :] = jnp.zeros((NT, HALO, 128), F32)
    v_s[:, 0:HALO, :] = jnp.zeros((NT, HALO, 128), F32)
    awo_u[:, D // 2:, :] = jnp.zeros((NT, PAD, 128), U32)
    tmpb[:, D:, :] = jnp.zeros((NT, PAD, 128), F32)
    tmpz[D:, :] = jnp.zeros((PAD, 128), F32)
    for c in range(NT):
        wait(*d_first[c])
        if c == 0:
            d_bxr.start()
        if c == 1:
            for d in d_rest:
                d.start()
        for b in range(NF):
            if c < 3:
                b_k_first(b, c, c + 1)
            elif b >= 2:
                b_k_first(b, c, c + 1, 128)
            elif c == 4:
                b_k_first(b, 3, 5)
    wkt[...] = _u32(bwqkv[:, D:2 * D].T)
    b_g(0)
    for p in range(1, NF // 2):
        b_g(p, {8: _fold(_f32(wkt[...]))})
    wait(d_bxr)
    for p in range(NF // 2, 4):
        for t in range(4):
            b_k(4 * p + t)
        if p == 3:
            b_fin_z(_perm_tables())
        b_g(p, None, 0, NT if p < 3 else G3_SPLIT)
    wait(*d_rest)
    tables = _perm_tables()
    permute_weight_cols(tables, bwqkv, 0, bwqp, 0)
    for sec in (2, 1, 0):
        dep_q = permute_weight_cols(tables, awqkv, sec * D, awp, sec * D)
    b_g(3, None, G3_SPLIT, NT)
    b_q(0)
    b_fin_kv()

    for i in range(NB):
        if i == 0:
            a_proj(0, 2, {24: dep_q, **{3 + 4 * c: repack_wo(c) for c in range(NT)}})
            b_fin_m()
            a_proj(0, 1, {4 + 2 * dp: permute_wo_rows(dp) for dp in range(DH // 2)})
            a_proj(0, 0)
        else:
            a_proj(i, 2)
            a_proj(i, 1)
            a_proj(i, 0, {4 + d: permute_m_rows(d) for d in range(DH)} if i == 1 else None)
        if i + 1 < NB:
            b_q(i + 1)
        for g in range(NG):
            group(i, g)
        if i >= 2:
            b_out(rows(i - 2))
        if i >= 1:
            a_out(rows(i - 1))
    b_out(rows(NB - 2))
    b_out(rows(NB - 1))
    a_out(slice(S - TM, S - 128))
    a_out(slice(S - 128, S - 64))
    a_out(slice(S - 64, S))

    wait(*outs)


@jax.jit
def pallas_concat_heads__sliding_local_dilated__linear_attn_block__prompt_kernel(
    A_x, A_wqkv, A_wo, B_x, B_wqkv, B_wo,
):
    def bf(*shape):
        return pltpu.VMEM(shape, BF16)

    def f32(*shape):
        return pltpu.VMEM(shape, F32)

    def packed(r, c):
        return pltpu.VMEM((r // 2, c), U32)

    any_spec = pl.BlockSpec(memory_space=pl.ANY)
    out = pl.pallas_call(
        _kernel,
        in_specs=[any_spec] * 6,
        out_specs=any_spec,
        out_shape=jax.ShapeDtypeStruct((S, 2 * D), BF16),
        scratch_shapes=[
            bf(S, D), bf(S, D), bf(D, 3 * D), bf(D, D), bf(D, 3 * D), bf(D, D),
            packed(D, 3 * D), pltpu.VMEM((NT, D // 2 + PAD, 128), U32), packed(D, D), packed(D, D), packed(D, D),
            packed(D, D), f32(NT, D + PAD, 128), f32(D + PAD, 128),
            f32(NT, S, 128), f32(NT, S + HALO, 128), f32(NT, S + HALO, 128), bf(NT, S, 128),
            f32(D, D), f32(NT, 8, 128), f32(NT, S, 128), bf(NT, S, 128), packed(D, S),
            bf(S, D), bf(S, D),
            pltpu.SemaphoreType.DMA((7,)),
        ],
        compiler_params=pltpu.CompilerParams(vmem_limit_bytes=100 * 2**20),
        name="fused_ab",
    )(A_x.reshape(S, D), A_wqkv, A_wo, B_x.reshape(S, D), B_wqkv, B_wo)
    return out.reshape(1, S, 2 * D)
```
